```python
import os as _os
_os.environ.setdefault("JAX_PLATFORMS", "cpu")
import jax
import jax.numpy as jnp

def _softmax(x, axis=-1):
    return jax.nn.softmax(x, axis=axis)
def _gelu(x):
    return jax.nn.gelu(x, approximate=True)
def _silu(x):
    return jax.nn.silu(x)
def _sigmoid(x):
    return jax.nn.sigmoid(x)
def _layernorm(x, axis=-1, eps=1e-5):
    m = jnp.mean(x, axis=axis, keepdims=True)
    v = jnp.var(x, axis=axis, keepdims=True)
    return (x - m) / jnp.sqrt(v + eps)
def _scatter_add(tgt, idx, src, axis=0):
    return tgt.at[idx].add(src)
def _segment_sum(src, seg, n):
    return jax.ops.segment_sum(src, seg, n)
class _Rng:
    def __init__(self, key):
        self._k = key
    def _next(self):
        self._k, sub = jax.random.split(self._k)
        return sub
    def normal(self, shape):
        return jax.random.normal(self._next(), shape, dtype=jnp.bfloat16)
    def randint(self, lo, hi, shape):
        return jax.random.randint(self._next(), shape, lo, hi, dtype=jnp.int32)
    def uniform(self, shape, lo=0.0, hi=1.0):
        return jax.random.uniform(self._next(), shape, jnp.bfloat16, lo, hi)
    def permutation(self, n):
        return jax.random.permutation(self._next(), n)


kernel_name = 'gated_mix__compressed_kv_cla__linear_attn_block__prompt'

def setup_inputs():
    _rng = _Rng(jax.random.key(int.from_bytes(__import__("os").urandom(4), "little")))
    _w = (lambda a: (lambda t: t.astype(jnp.bfloat16) if jnp.issubdtype(t.dtype, jnp.floating) else t)(jnp.asarray(a)))
    def _A_setup():
        B, H, Sq, Sk, D, M = 1, 16, 2048, 2048, 256, 448
        Dc = 4 * D
        return {
            "x": _w((lambda *s: _rng.normal(s) * 0.05)(B, Sq, M)),
            "c_kv": _w((lambda *s: _rng.normal(s) * 0.8)(B, Sk, Dc)),
            "w_q": _w((lambda *s: _rng.normal(s) * 3.2)(M, H, D) * (M ** -0.5)),
            "w_uk": _w((lambda *s: _rng.normal(s) * 3.2)(Dc, H, D) * (Dc ** -0.5)),
            "w_uv": _w((lambda *s: _rng.normal(s) * 0.8)(Dc, H, D) * (Dc ** -0.5)),
            "w_o": _w((lambda *s: _rng.normal(s) * 0.8)(H, D, M) * ((H * D) ** -0.5)),
        }
    _A_in = _A_setup()

    def _B_setup():
        B, S, D = 1, 2048, 448
        return {
            "x": _w((lambda *s: _rng.normal(s) * 0.05)(B, S, D)),
            "wqkv": _w((lambda *s: _rng.normal(s) * 1.6)(D, 3 * D)),
            "wo": _w((lambda *s: _rng.normal(s) * 0.4)(D, D)),
        }
    _B_in = _B_setup()

    return {
        "A_x": _A_in["x"],
        "A_c_kv": _A_in["c_kv"],
        "A_w_q": _A_in["w_q"],
        "A_w_uk": _A_in["w_uk"],
        "A_w_uv": _A_in["w_uv"],
        "A_w_o": _A_in["w_o"],
        "B_x": _B_in["x"],
        "B_wqkv": _B_in["wqkv"],
        "B_wo": _B_in["wo"],
        "gate_w": _w((lambda *s: _rng.normal(s) * 0.05)(448) * 16.0),
    }

def reference(A_x, A_c_kv, A_w_q, A_w_uk, A_w_uv, A_w_o, B_x, B_wqkv, B_wo, gate_w):
    def _A_ref(x, c_kv, w_q, w_uk, w_uv, w_o):
        B, Sq, M = x.shape[0], x.shape[1], x.shape[2]
        Sk = c_kv.shape[1]
        H, D = w_q.shape[1], w_q.shape[2]
        q = jnp.einsum("bqm,mhd->bhqd", x, w_q)
        k = jnp.einsum("bkc,chd->bhkd", c_kv, w_uk)
        v = jnp.einsum("bkc,chd->bhkd", c_kv, w_uv)
        scores = jnp.einsum("bhqd,bhkd->bhqk", q, k) * (D ** -0.5)
        off = Sk - Sq
        qi = jnp.arange(Sq)[:, None]
        kj = jnp.arange(Sk)[None, :]
        cmask = kj <= (qi + off)
        scores = jnp.where(cmask[None, None], scores, -1e9)
        p = _softmax(scores, axis=-1)
        ctx = jnp.einsum("bhqk,bhkd->bhqd", p, v)
        return jnp.einsum("bhqd,hdm->bqm", ctx, w_o)

    def _B_ref(x, wqkv, wo):
        B, S, D = x.shape
        H = 16; Dh = D // H
        qkv = (lambda x, *d: x.transpose(*d))((x @ wqkv).reshape(B, S, 3, H, Dh), 2, 0, 3, 1, 4)
        q, k, v = qkv[0], qkv[1], qkv[2]
        phi = lambda t: jnp.where(t > 0, t + 1, jnp.exp(t)) + 1e-6
        pq, pk = phi(q), phi(k)
        kv = jnp.einsum("bhsd,bhse->bhde", pk, v)
        z = jnp.einsum("bhsd->bhd", pk)
        num = jnp.einsum("bhqd,bhde->bhqe", pq, kv)
        den = jnp.einsum("bhqd,bhd->bhq", pq, z)[..., None] + 1e-6
        o = num / den
        return (lambda x, *d: x.transpose(*d))(o, 0, 2, 1, 3).reshape(B, S, D) @ wo

    x = A_x
    g = _sigmoid((x * gate_w).sum(-1, keepdims=True))
    a = _A_ref(x, A_c_kv, A_w_q, A_w_uk, A_w_uv, A_w_o)
    b = _B_ref(x, B_wqkv, B_wo)
    return g * a + (1 - g) * b
```

```python
import functools
import jax
import jax.numpy as jnp
from jax import lax
import jax.experimental.pallas as pl
import jax.experimental.pallas.tpu as pltpu

NT = (((1,), (1,)), ((), ()))
BF = jnp.bfloat16
F32 = jnp.float32
U32 = jnp.uint32


def _dot(a, b):
    return jnp.dot(a, b, preferred_element_type=F32)


def _dot_nt(a, b):
    return lax.dot_general(a, b, NT, preferred_element_type=F32)


def _phi(t):
    return jnp.where(t > 0, t + 1.0, jnp.exp(t)) + 1e-6


def _kernel(xT_ref, wqkv_ref, bwo_ref, gw_ref, woT_ref, c_hbm, wq_hbm, wuk_hbm, wuv_hbm,
            oT_ref,
            c_sc, raw_q, raw_k, raw_v, pk_q, pk_k, pk_v, ext_q, ext_k, ext_v,
            x_sc, q_sc, k_sc, v_sc, acc_sc, g_sc, wT_sc, bwoT_sc, pqT_sc, gT_sc, kvT_sc, lhs_sc, sems,
            *, T, H, S, D, M, Dc, HB, TB):
    h = pl.program_id(0)
    scale = D ** -0.5
    Dh = M // HB
    n_t = pl.cdiv(M, 128)

    weights = ((wq_hbm, raw_q, pk_q, ext_q, M), (wuk_hbm, raw_k, pk_k, ext_k, Dc), (wuv_hbm, raw_v, pk_v, ext_v, Dc))

    def extract(hd):
        j = hd // 2
        sh = ((hd % 2) * 16).astype(U32)
        for (_, _, pk, ext, C) in weights:
            for half in range(D // 128):
                a = pk[0, half, pl.ds(j, C // 2, stride=8), :]
                b = pk[1, half, pl.ds(j, C // 2, stride=8), :]
                r = ((a >> sh) & U32(0xFFFF)) | ((b << (U32(16) - sh)) & U32(0xFFFF0000))
                ext[:, half * 128:(half + 1) * 128] = r

    def trange(t):
        c0, c1 = t * 128, min((t + 1) * 128, M)
        h0, h1 = c0 // Dh, (c1 - 1) // Dh
        r0, r1 = h0 * Dh, (h1 + 1) * Dh
        return c0, c1, (r0 // 16) * 16, min(-(-r1 // 16) * 16, M)

    @pl.when(h == 0)
    def _init():
        copies = [pltpu.make_async_copy(c_hbm, c_sc, sems.at[0])]
        for n, (w_hbm, raw, _, _, _) in enumerate(weights):
            copies.append(pltpu.make_async_copy(w_hbm, raw, sems.at[1 + n]))
        for cp in copies:
            cp.start()

        wT_sc[0:3 * M, :] = wqkv_ref[...].T
        wT_sc[3 * M:3 * M + 16, :] = jnp.broadcast_to(gw_ref[...], (16, M))
        bwoT_sc[...] = bwo_ref[...].T
        kvT_sc[...] = jnp.zeros_like(kvT_sc)
        ones = jnp.ones((16, TB), BF)
        gw = gw_ref[...].astype(F32)

        def b1(i, carry):
            r = pl.multiple_of(i * TB, TB)
            xTc = xT_ref[:, pl.ds(r, TB)]
            qkvT = _dot(wT_sc[...], xTc)
            pqT_sc[:, pl.ds(r, TB)] = _phi(qkvT[:M]).astype(BF)
            pkT = _phi(qkvT[M:2 * M]).astype(BF)
            vT = qkvT[2 * M:3 * M].astype(BF)
            gT_sc[:, pl.ds(r, TB)] = qkvT[3 * M:3 * M + 8]
            for t in range(n_t):
                c0, c1, r0, r1 = trange(t)
                lhs = jnp.concatenate([vT[r0:r1], ones], axis=0)
                res = _dot_nt(lhs, pkT[c0:c1])
                kvT_sc[r0:r1, c0:c1] += res[:r1 - r0]
                kvT_sc[M:M + 16, c0:c1] += res[r1 - r0:]
            xc = xTc.T
            x_sc[pl.ds(r, TB), :] = xc
            g_sc[pl.ds(r, TB), :] = jax.nn.sigmoid(
                jnp.sum(xc.astype(F32) * gw, axis=-1, keepdims=True))
            return carry

        lax.fori_loop(0, S // TB, b1, 0)

        ri = lax.broadcasted_iota(jnp.int32, (M, M), 0) // Dh
        ci = lax.broadcasted_iota(jnp.int32, (M, M), 1) // Dh
        bd = ri == ci
        lhs_sc[0] = jnp.where(bd, kvT_sc[0:M, :], 0.0).astype(BF)
        lhs_sc[1] = jnp.where(bd, kvT_sc[M:M + 1, :], 0.0).astype(BF)

        def b3(i, carry):
            r = pl.multiple_of(i * TB, TB)
            pqT = pqT_sc[:, pl.ds(r, TB)]
            parts = []
            for t in range(n_t):
                c0, c1, r0, r1 = trange(t)
                lhs = jnp.concatenate([lhs_sc[0, r0:r1, c0:c1], lhs_sc[1, r0:r1, c0:c1]], axis=0)
                res = _dot(lhs, pqT[c0:c1])
                parts.append((r0, r1, res[:r1 - r0], res[r1 - r0:]))
            o_rows = []
            bounds = sorted(set([p[0] for p in parts] + [p[1] for p in parts]))
            for a, b in zip(bounds[:-1], bounds[1:]):
                num = den = None
                for (r0, r1, n_, d_) in parts:
                    if r0 <= a and b <= r1:
                        nn, dd = n_[a - r0:b - r0], d_[a - r0:b - r0]
                        num = nn if num is None else num + nn
                        den = dd if den is None else den + dd
                o_rows.append((num / (den + 1e-6)).astype(BF))
            oT = jnp.concatenate(o_rows, axis=0)
            bT = _dot(bwoT_sc[...], oT)
            gT = jax.nn.sigmoid(gT_sc[0:1, pl.ds(r, TB)])
            acc_sc[:, pl.ds(r, TB)] = (1.0 - gT) * bT
            return carry

        lax.fori_loop(0, S // TB, b3, 0)

        for cp in copies:
            cp.wait()

        CH = 64
        for (_, raw, pk, _, C) in weights:
            def rp(i, carry, raw=raw, pk=pk):
                r = pl.multiple_of(i * CH, CH)
                u = pltpu.bitcast(raw[pl.ds(r, CH), :, :], U32)
                u = u.reshape(CH // 2, 2, H // 2, D)
                ro = pl.multiple_of(i * (CH * 4), CH * 4)
                for par in range(2):
                    for half in range(D // 128):
                        pk[par, half, pl.ds(ro, CH * 4), :] = (
                            u[:, par, :, half * 128:(half + 1) * 128].reshape(CH * 4, 128))
                return carry
            lax.fori_loop(0, C // CH, rp, 0)
        extract(h)

    woT = woT_ref[...]
    nq = S // T
    HT = T // 2
    row = lax.broadcasted_iota(jnp.int32, (HT, HT), 0)
    col = lax.broadcasted_iota(jnp.int32, (HT, HT), 1)
    tri = col <= row
    qs, ks, vs, ss = {}, {}, {}, {}

    def P(i):
        r0 = i * T
        cch = c_sc[r0:r0 + T, :]
        qs[i] = (_dot(x_sc[r0:r0 + T, :], pltpu.bitcast(ext_q[...], BF)) * scale).astype(BF)
        ks[i] = _dot(cch, pltpu.bitcast(ext_k[...], BF)).astype(BF)
        vs[i] = _dot(cch, pltpu.bitcast(ext_v[...], BF)).astype(BF)

    CK = 512
    LAG = 1

    state = {}

    def kcat(d, a, b):
        parts = []
        t = a // T
        while t * T < b:
            lo, hi = max(a, t * T) - t * T, min(b, (t + 1) * T) - t * T
            parts.append(d[t][lo:hi])
            t += 1
        return jnp.concatenate(parts, axis=0) if len(parts) > 1 else parts[0]

    def S_(i, a, b):
        r0 = i * T
        q = qs[i]
        if b == r0 + T:
            sm = _dot_nt(q, kcat(ks, a, r0 + HT))
            sr = _dot_nt(q[HT:], ks[i][HT:])
            state[(i, a)] = (sm, sr)
        else:
            state[(i, a)] = (_dot_nt(q, kcat(ks, a, b)), None)

    def V_(i, a, b):
        r0 = i * T
        sm, sr = state.pop((i, a))
        if sr is not None:
            w = sm.shape[1]
            dt = jnp.where(tri, sm[:HT, w - HT:], -1e9)
            st = jnp.concatenate([sm[:HT, :w - HT], dt], axis=1) if w > HT else dt
            sb = jnp.concatenate([sm[HT:], jnp.where(tri, sr, -1e9)], axis=1)
            mt = jnp.max(st, axis=-1, keepdims=True)
            mb = jnp.max(sb, axis=-1, keepdims=True)
            pt = jnp.exp(st - mt)
            pb = jnp.exp(sb - mb)
            m = jnp.concatenate([mt, mb], axis=0)
            l = jnp.concatenate([jnp.sum(pt, axis=-1, keepdims=True), jnp.sum(pb, axis=-1, keepdims=True)], axis=0)
            pb = pb.astype(BF)
            pm = jnp.concatenate([pt.astype(BF), pb[:, :w]], axis=0)
            ctx = _dot(pm, kcat(vs, a, r0 + HT))
            ctx_r = _dot(pb[:, w:], vs[i][HT:])
            ctx = jnp.concatenate([ctx[:HT], ctx[HT:] + ctx_r], axis=0)
        else:
            m = jnp.max(sm, axis=-1, keepdims=True)
            p = jnp.exp(sm - m)
            l = jnp.sum(p, axis=-1, keepdims=True)
            ctx = _dot(p.astype(BF), kcat(vs, a, b))
        state.setdefault(('acc', i), []).append((m, l, ctx))

    def O_(i):
        r0 = i * T
        parts = state.pop(('acc', i))
        m = parts[0][0]
        for (mc, _, _) in parts[1:]:
            m = jnp.maximum(m, mc)
        if len(parts) == 1:
            l = parts[0][1]
            rr = g_sc[r0:r0 + T, :] / l
            ctx = parts[0][2] * rr
        else:
            es = [jnp.exp(mc - m) for (mc, _, _) in parts]
            l = sum(e * lc for e, (_, lc, _) in zip(es, parts))
            rr = g_sc[r0:r0 + T, :] / l
            ctx = sum((e * rr) * cx for e, (_, _, cx) in zip(es, parts))
        acc_sc[:, r0:r0 + T] += _dot_nt(woT, ctx.astype(BF))

    items = []
    for i in range(nq):
        items.append(('P', i))
        end = (i + 1) * T
        bnds = list(range(0, end, CK)) + [end]
        for a, b in zip(bnds[:-1], bnds[1:]):
            items.append(('S', i, a, b))
    OLAG = 1
    out = []
    pending = []
    pend_o = []
    def emit(x):
        nonlocal pend_o
        out.append(x)
        if x[0] in ('S', 'P', 'V'):
            pend_o = [(c + 1, y) for (c, y) in pend_o]
            while pend_o and pend_o[0][0] >= OLAG:
                out.append(pend_o.pop(0)[1])
    for it in items:
        emit(it)
        pending = [(c + 1, x) for (c, x) in pending]
        if it[0] == 'S':
            pending.append((0, it))
        while pending and pending[0][0] >= LAG:
            _, x = pending.pop(0)
            emit(('V',) + x[1:])
            if x[3] == (x[1] + 1) * T:
                if OLAG == 0:
                    out.append(('O', x[1]))
                else:
                    pend_o.append((0, ('O', x[1])))
    for (_, x) in pending:
        emit(('V',) + x[1:])
        if x[3] == (x[1] + 1) * T:
            pend_o.append((0, ('O', x[1])))
    for (_, y) in pend_o:
        out.append(y)
    for it in out:
        {'P': P, 'S': S_, 'V': V_, 'O': O_}[it[0]](*it[1:])

    extract(jnp.minimum(h + 1, H - 1))

    @pl.when(h == H - 1)
    def _():
        oT_ref[...] = acc_sc[...].astype(oT_ref.dtype)


@jax.jit
def pallas_gated_mix__compressed_kv_cla__linear_attn_block__prompt_kernel(
    A_x, A_c_kv, A_w_q, A_w_uk, A_w_uv, A_w_o, B_x, B_wqkv, B_wo, gate_w):
    B, S, M = A_x.shape
    Dc = A_c_kv.shape[2]
    H, D = A_w_q.shape[1], A_w_q.shape[2]
    T = 256
    TB = 512
    HB = 16
    xT = jnp.swapaxes(A_x, 1, 2).reshape(M, S)
    woT = jnp.swapaxes(A_w_o, 1, 2)
    c = A_c_kv.reshape(S, Dc)
    gw = gate_w.reshape(1, M)
    kern = functools.partial(_kernel, T=T, H=H, S=S, D=D, M=M, Dc=Dc, HB=HB, TB=TB)
    hbm_spec = pl.BlockSpec(memory_space=pltpu.HBM)
    outT = pl.pallas_call(
        kern,
        grid=(H,),
        in_specs=[
            pl.BlockSpec((M, S), lambda h: (0, 0)),
            pl.BlockSpec((M, 3 * M), lambda h: (0, 0)),
            pl.BlockSpec((M, M), lambda h: (0, 0)),
            pl.BlockSpec((1, M), lambda h: (0, 0)),
            pl.BlockSpec((None, M, D), lambda h: (h, 0, 0)),
            hbm_spec, hbm_spec, hbm_spec, hbm_spec,
        ],
        out_specs=pl.BlockSpec((M, S), lambda h: (0, 0)),
        out_shape=jax.ShapeDtypeStruct((M, S), BF),
        scratch_shapes=[
            pltpu.VMEM((S, Dc), BF),
            pltpu.VMEM((M, H, D), BF),
            pltpu.VMEM((Dc, H, D), BF),
            pltpu.VMEM((Dc, H, D), BF),
            pltpu.VMEM((2, D // 128, M * 4, 128), U32),
            pltpu.VMEM((2, D // 128, Dc * 4, 128), U32),
            pltpu.VMEM((2, D // 128, Dc * 4, 128), U32),
            pltpu.VMEM((M // 2, D), U32),
            pltpu.VMEM((Dc // 2, D), U32),
            pltpu.VMEM((Dc // 2, D), U32),
            pltpu.VMEM((S, M), BF),
            pltpu.VMEM((S, D), BF),
            pltpu.VMEM((S, D), BF),
            pltpu.VMEM((S, D), BF),
            pltpu.VMEM((M, S), F32),
            pltpu.VMEM((S, 1), F32),
            pltpu.VMEM((3 * M + 16, M), BF),
            pltpu.VMEM((M, M), BF),
            pltpu.VMEM((M, S), BF),
            pltpu.VMEM((8, S), F32),
            pltpu.VMEM((M + 16, M), F32),
            pltpu.VMEM((2, M, M), BF),
            pltpu.SemaphoreType.DMA((4,)),
        ],
        compiler_params=pltpu.CompilerParams(
            dimension_semantics=("arbitrary",),
            vmem_limit_bytes=110 * 1024 * 1024),
    )(xT, B_wqkv, B_wo, gw, woT, c, A_w_q, A_w_uk, A_w_uv)
    return jnp.swapaxes(outT.reshape(B, M, S), 1, 2)
```

```python
import functools

import jax
import jax.numpy as jnp
from jax import lax
import jax.experimental.pallas as pl
import jax.experimental.pallas.tpu as pltpu

NT = (((1,), (1,)), ((), ()))
BF = jnp.bfloat16
F32 = jnp.float32
U32 = jnp.uint32


def _dot(a, b):
    return jnp.dot(a, b, preferred_element_type=F32)


def _dot_nt(a, b):
    return lax.dot_general(a, b, NT, preferred_element_type=F32)


def _phi(t):
    return jnp.where(t > 0, t + 1.0, jnp.exp(t)) + 1e-6


def _kernel(gw_hbm, woT_hbm, xT_hbm, wqkv_hbm, bwo_hbm, c_hbm, wq_hbm, wuk_hbm, wuv_hbm,
            oT_hbm,
            xT_sc, wqkv_sc, bwo_sc, c_sc,
            raw_q0, raw_k0, raw_v0, raw_q1, raw_k1, raw_v1,
            pk_q, pk_k, pk_v, ext_q, ext_k, ext_v,
            x_sc, acc_sc, g_sc, wT_sc, bwoT_sc, pqT_sc, gT_sc, kvT_sc, lhs_sc, o_sc, gw_sc, woT_sc,
            sems, osems,
            *, T, H, S, D, M, Dc, HB, TB, CK, AORD, NLATE):
    h = pl.program_id(0)
    scale = D ** -0.5
    Dh = M // HB
    n_t = pl.cdiv(M, 128)
    HG = 8
    PR = HG // 2

    weights = ((wq_hbm, (raw_q0, raw_q1), pk_q, ext_q, M),
               (wuk_hbm, (raw_k0, raw_k1), pk_k, ext_k, Dc),
               (wuv_hbm, (raw_v0, raw_v1), pk_v, ext_v, Dc))

    def w_copy(n, g):
        w_hbm, raws = weights[n][0], weights[n][1]
        return pltpu.make_async_copy(w_hbm.at[:, pl.ds(g * HG, HG), :], raws[g],
                                     sems.at[6 + 3 * g + n])

    def o_copy(i):
        return pltpu.make_async_copy(o_sc.at[:, pl.ds(i * T, T)], oT_hbm.at[:, pl.ds(i * T, T)],
                                     osems.at[i])

    def repack(g):
        CH = 64
        for (_, raws, pk, _, C) in weights:
            def rp(i, carry, raw=raws[g], pk=pk):
                r = pl.multiple_of(i * CH, CH)
                v = raw[pl.ds(r, CH), :, :].reshape(CH // 2, 2 * HG, D)
                u = pltpu.bitcast(v, U32)
                n = CH * PR
                ro = pl.multiple_of(i * n, n)
                for half in range(D // 128):
                    pk[g, half, pl.ds(ro, n), :] = u[:, :, half * 128:(half + 1) * 128].reshape(n, 128)
                return carry
            lax.fori_loop(0, C // CH, rp, 0)

    def extract(hd):
        g = hd // HG
        j = (hd % HG) // 2
        sh = ((hd % 2) * 16).astype(U32)
        for (_, _, pk, ext, C) in weights:
            for half in range(D // 128):
                a = pk[g, half, pl.ds(j, C // 2, stride=2 * PR), :]
                b = pk[g, half, pl.ds(j + PR, C // 2, stride=2 * PR), :]
                r = ((a >> sh) & U32(0xFFFF)) | ((b << (U32(16) - sh)) & U32(0xFFFF0000))
                ext[:, half * 128:(half + 1) * 128] = r

    def trange(t):
        c0, c1 = t * 128, min((t + 1) * 128, M)
        h0, h1 = c0 // Dh, (c1 - 1) // Dh
        r0, r1 = h0 * Dh, (h1 + 1) * Dh
        return c0, c1, (r0 // 16) * 16, min(-(-r1 // 16) * 16, M)

    @pl.when(h == 0)
    def _init():
        cp_wqkv = pltpu.make_async_copy(wqkv_hbm, wqkv_sc, sems.at[0])
        cp_x = pltpu.make_async_copy(xT_hbm, xT_sc, sems.at[1])
        cp_bwo = pltpu.make_async_copy(bwo_hbm, bwo_sc, sems.at[2])
        cp_c = pltpu.make_async_copy(c_hbm, c_sc, sems.at[3])
        cp_gw = pltpu.make_async_copy(gw_hbm, gw_sc, sems.at[4])
        cp_wo = pltpu.make_async_copy(woT_hbm, woT_sc, sems.at[5])
        cp_wqkv.start()
        cp_gw.start()
        cp_x.start()
        cp_bwo.start()

        kvT_sc[...] = jnp.zeros_like(kvT_sc)
        cp_wqkv.wait()
        cp_c.start()
        for n in range(3):
            w_copy(n, 0).start()
        cp_wo.start()
        cp_gw.wait()
        gw_row = gw_sc[...].reshape(1, M)
        wT_sc[3 * M:3 * M + 16, :] = jnp.broadcast_to(gw_row, (16, M))
        wT_sc[0:3 * M, :] = wqkv_sc[...].T
        cp_bwo.wait()
        bwoT_sc[...] = bwo_sc[...].T
        ones = jnp.ones((16, TB), BF)
        gw = gw_row.astype(F32)
        cp_x.wait()

        def b1(i, carry):
            r = pl.multiple_of(i * TB, TB)
            xTc = xT_sc[:, pl.ds(r, TB)]
            qkvT = _dot(wT_sc[...], xTc)
            pqT_sc[:, pl.ds(r, TB)] = _phi(qkvT[:M]).astype(BF)
            pkT = _phi(qkvT[M:2 * M]).astype(BF)
            vT = qkvT[2 * M:3 * M].astype(BF)
            gT_sc[:, pl.ds(r, TB)] = qkvT[3 * M:3 * M + 8]
            for t in range(n_t):
                c0, c1, r0, r1 = trange(t)
                lhs = jnp.concatenate([vT[r0:r1], ones], axis=0)
                res = _dot_nt(lhs, pkT[c0:c1])
                kvT_sc[r0:r1, c0:c1] += res[:r1 - r0]
                kvT_sc[M:M + 16, c0:c1] += res[r1 - r0:]
            xc = xTc.T
            x_sc[pl.ds(r, TB), :] = xc
            g_sc[pl.ds(r, TB), :] = jax.nn.sigmoid(
                jnp.sum(xc.astype(F32) * gw, axis=-1, keepdims=True))
            return carry

        lax.fori_loop(0, S // TB, b1, 0)

        for n in range(3):
            w_copy(n, 1).start()
        ri = lax.broadcasted_iota(jnp.int32, (M, M), 0) // Dh
        ci = lax.broadcasted_iota(jnp.int32, (M, M), 1) // Dh
        lhs_sc[0:M, :] = jnp.where(ri == ci, kvT_sc[0:M, :], 0.0).astype(BF)
        hr = lax.broadcasted_iota(jnp.int32, (HB, M), 0)
        hc = lax.broadcasted_iota(jnp.int32, (HB, M), 1) // Dh
        lhs_sc[M:M + HB, :] = jnp.where(hr == hc, kvT_sc[M:M + HB, :], 0.0).astype(BF)

        sub8 = lax.broadcasted_iota(jnp.int32, (8, TB), 0)

        def nd(r):
            pqT = pqT_sc[:, r:r + TB]
            parts = []
            den = None
            for t in range(n_t):
                c0, c1, r0, r1 = trange(t)
                lhs = jnp.concatenate([lhs_sc[r0:r1, c0:c1], lhs_sc[M:M + HB, c0:c1]], axis=0)
                res = _dot(lhs, pqT[c0:c1])
                parts.append((r0, r1, res[:r1 - r0]))
                den = res[r1 - r0:] if den is None else den + res[r1 - r0:]
            return parts, den

        def fin(r, pd):
            parts, den = pd
            rec = 1.0 / (den + 1e-6)
            o_rows = []
            for a in range(0, M, 8):
                num = None
                for (r0, r1, n_) in parts:
                    if r0 <= a < r1:
                        nn = n_[a - r0:a - r0 + 8]
                        num = nn if num is None else num + nn
                h1, h2 = a // Dh, (a + 7) // Dh
                rr = jnp.broadcast_to(rec[h1:h1 + 1], (8, TB))
                if h2 != h1:
                    rr = jnp.where(sub8 < h2 * Dh - a, rr, jnp.broadcast_to(rec[h2:h2 + 1], (8, TB)))
                o_rows.append(num * rr)
            oT = jnp.concatenate(o_rows, axis=0).astype(BF)
            bT = _dot(bwoT_sc[...], oT)
            gT = jax.nn.sigmoid(gT_sc[0:1, r:r + TB])
            acc_sc[:, r:r + TB] = (1.0 - gT) * bT

        prev = None
        for u in range(S // TB):
            cur = nd(u * TB)
            if prev is not None:
                fin((u - 1) * TB, prev)
            prev = cur
        fin(S - TB, prev)

        cp_c.wait()
        for n in range(3):
            w_copy(n, 0).wait()
        cp_wo.wait()
        repack(0)
        extract(h)

    @pl.when(h == 1)
    def _():
        for n in range(3):
            w_copy(n, 1).wait()
        repack(1)

    woT = woT_sc[h]
    HT = T // 2
    row = lax.broadcasted_iota(jnp.int32, (HT, HT), 0)
    col = lax.broadcasted_iota(jnp.int32, (HT, HT), 1)
    tri = col <= row
    qs, ks, vs = {}, {}, {}
    state = {}

    def P_(i):
        r0 = i * T
        cch = c_sc[r0:r0 + T, :]
        qs[i] = (_dot(x_sc[r0:r0 + T, :], pltpu.bitcast(ext_q[...], BF)) * scale).astype(BF)
        ks[i] = _dot(cch, pltpu.bitcast(ext_k[...], BF)).astype(BF)
        vs[i] = _dot(cch, pltpu.bitcast(ext_v[...], BF)).astype(BF)

    def kcat(d, a, b):
        parts = []
        t = a // T
        while t * T < b:
            lo, hi = max(a, t * T) - t * T, min(b, (t + 1) * T) - t * T
            parts.append(d[t][lo:hi])
            t += 1
        return jnp.concatenate(parts, axis=0) if len(parts) > 1 else parts[0]

    def S_(i, a, b):
        r0 = i * T
        q = qs[i]
        if b == r0 + T:
            sm = _dot_nt(q, kcat(ks, a, r0 + HT))
            sr = _dot_nt(q[HT:], ks[i][HT:])
            state[(i, a)] = (sm, sr)
        else:
            state[(i, a)] = (_dot_nt(q, kcat(ks, a, b)), None)

    def V_(i, a, b):
        r0 = i * T
        sm, sr = state.pop((i, a))
        if sr is not None:
            w = sm.shape[1]
            dt = jnp.where(tri, sm[:HT, w - HT:], -1e9)
            st = jnp.concatenate([sm[:HT, :w - HT], dt], axis=1) if w > HT else dt
            sb = jnp.concatenate([sm[HT:], jnp.where(tri, sr, -1e9)], axis=1)
            mt = jnp.max(st, axis=-1, keepdims=True)
            mb = jnp.max(sb, axis=-1, keepdims=True)
            pt = jnp.exp(st - mt)
            pb = jnp.exp(sb - mb)
            m = jnp.concatenate([mt, mb], axis=0)
            l = jnp.concatenate([jnp.sum(pt, axis=-1, keepdims=True),
                                 jnp.sum(pb, axis=-1, keepdims=True)], axis=0)
            pb = pb.astype(BF)
            pm = jnp.concatenate([pt.astype(BF), pb[:, :w]], axis=0)
            ctx = _dot(pm, kcat(vs, a, r0 + HT))
            ctx_r = _dot(pb[:, w:], vs[i][HT:])
            ctx = jnp.concatenate([ctx[:HT], ctx[HT:] + ctx_r], axis=0)
        else:
            m = jnp.max(sm, axis=-1, keepdims=True)
            p = jnp.exp(sm - m)
            l = jnp.sum(p, axis=-1, keepdims=True)
            ctx = _dot(p.astype(BF), kcat(vs, a, b))
        state.setdefault(('acc', i), []).append((m, l, ctx))

    def O_(i):
        r0 = i * T
        parts = state.pop(('acc', i))
        m = parts[0][0]
        for (mc, _, _) in parts[1:]:
            m = jnp.maximum(m, mc)
        if len(parts) == 1:
            rr = g_sc[r0:r0 + T, :] / parts[0][1]
            ctx = parts[0][2] * rr
        else:
            es = [jnp.exp(mc - m) for (mc, _, _) in parts]
            l = sum(e * lc for e, (_, lc, _) in zip(es, parts))
            rr = g_sc[r0:r0 + T, :] / l
            ctx = sum((e * rr) * cx for e, (_, _, cx) in zip(es, parts))
        a_new = acc_sc[:, r0:r0 + T] + _dot_nt(woT, ctx.astype(BF))
        acc_sc[:, r0:r0 + T] = a_new
        o_sc[:, r0:r0 + T] = a_new.astype(BF)
        if i not in AORD[-NLATE:]:
            o_copy(i).start()

    items = []
    donep = 0
    for i in AORD:
        while donep <= i:
            items.append(('P', donep))
            donep += 1
        end = (i + 1) * T
        bnds = list(range(0, end, CK)) + [end]
        for a, b in zip(bnds[:-1], bnds[1:]):
            items.append(('S', i, a, b))
    out = []
    pend_v = []
    pend_o = []

    def emit(x):
        out.append(x)
        if pend_o:
            out.append(pend_o.pop(0))

    def emit_v(x):
        emit(('V',) + x[1:])
        if x[3] == (x[1] + 1) * T:
            pend_o.append(('O', x[1]))

    for it in items:
        emit(it)
        if pend_v:
            emit_v(pend_v.pop(0))
        if it[0] == 'S':
            pend_v.append(it)
    while pend_v:
        emit_v(pend_v.pop(0))
    out.extend(pend_o)
    for it in out:
        {'P': P_, 'S': S_, 'V': V_, 'O': O_}[it[0]](*it[1:])

    extract(jnp.minimum(h + 1, H - 1))

    for i in AORD[:-NLATE]:
        o_copy(i).wait()

    @pl.when(h == H - 1)
    def _():
        for i in AORD[-NLATE:]:
            o_copy(i).start()
        for i in AORD[-NLATE:]:
            o_copy(i).wait()


@jax.jit
def pallas_gated_mix__compressed_kv_cla__linear_attn_block__prompt_kernel(
    A_x: jax.Array,
    A_c_kv: jax.Array,
    A_w_q: jax.Array,
    A_w_uk: jax.Array,
    A_w_uv: jax.Array,
    A_w_o: jax.Array,
    B_x: jax.Array,
    B_wqkv: jax.Array,
    B_wo: jax.Array,
    gate_w: jax.Array,
):
    B, S, M = A_x.shape
    Dc = A_c_kv.shape[2]
    H, D = A_w_q.shape[1], A_w_q.shape[2]
    assert B == 1 and A_c_kv.shape[1] == S and H == 16 and D == 256 and S == 2048
    T = 256
    TB = 512
    HB = 16
    CK = 512
    AORD = (1, 3, 4, 5, 6, 7, 2, 0)
    NLATE = 2
    xT = jnp.swapaxes(A_x, 1, 2).reshape(M, S)
    woT = jnp.swapaxes(A_w_o, 1, 2)
    c = A_c_kv.reshape(S, Dc)
    kern = functools.partial(_kernel, T=T, H=H, S=S, D=D, M=M, Dc=Dc, HB=HB, TB=TB, CK=CK,
                             AORD=AORD, NLATE=NLATE)
    hbm_spec = pl.BlockSpec(memory_space=pltpu.HBM)
    NG = H // 8
    outT = pl.pallas_call(
        kern,
        grid=(H,),
        in_specs=[hbm_spec] * 9,
        out_specs=hbm_spec,
        out_shape=jax.ShapeDtypeStruct((M, S), BF),
        scratch_shapes=[
            pltpu.VMEM((M, S), BF),
            pltpu.VMEM((M, 3 * M), BF),
            pltpu.VMEM((M, M), BF),
            pltpu.VMEM((S, Dc), BF),
            pltpu.VMEM((M, 8, D), BF),
            pltpu.VMEM((Dc, 8, D), BF),
            pltpu.VMEM((Dc, 8, D), BF),
            pltpu.VMEM((M, 8, D), BF),
            pltpu.VMEM((Dc, 8, D), BF),
            pltpu.VMEM((Dc, 8, D), BF),
            pltpu.VMEM((NG, D // 128, M * 4 + 8, 128), U32),
            pltpu.VMEM((NG, D // 128, Dc * 4 + 8, 128), U32),
            pltpu.VMEM((NG, D // 128, Dc * 4 + 8, 128), U32),
            pltpu.VMEM((M // 2, D), U32),
            pltpu.VMEM((Dc // 2, D), U32),
            pltpu.VMEM((Dc // 2, D), U32),
            pltpu.VMEM((S, M), BF),
            pltpu.VMEM((M, S), F32),
            pltpu.VMEM((S, 1), F32),
            pltpu.VMEM((3 * M + 16, M), BF),
            pltpu.VMEM((M, M), BF),
            pltpu.VMEM((M, S), BF),
            pltpu.VMEM((8, S), F32),
            pltpu.VMEM((M + 16, M), F32),
            pltpu.VMEM((M + HB, M), BF),
            pltpu.VMEM((M, S), BF),
            pltpu.VMEM((M,), BF),
            pltpu.VMEM((H, M, D), BF),
            pltpu.SemaphoreType.DMA((6 + 3 * NG,)),
            pltpu.SemaphoreType.DMA((S // T,)),
        ],
        compiler_params=pltpu.CompilerParams(
            dimension_semantics=("arbitrary",),
            vmem_limit_bytes=110 * 1024 * 1024),
    )(gate_w, woT, xT, B_wqkv, B_wo, c, A_w_q, A_w_uk, A_w_uv)
    return jnp.swapaxes(outT.reshape(B, M, S), 1, 2)
```

```python
import functools

import jax
import jax.numpy as jnp
from jax import lax
import jax.experimental.pallas as pl
import jax.experimental.pallas.tpu as pltpu

NT = (((1,), (1,)), ((), ()))
BF = jnp.bfloat16
F32 = jnp.float32
U32 = jnp.uint32


def _dot(a, b):
    return jnp.dot(a, b, preferred_element_type=F32)


def _dot_nt(a, b):
    return lax.dot_general(a, b, NT, preferred_element_type=F32)


def _phi(t):
    return jnp.where(t > 0, t + 1.0, jnp.exp(t)) + 1e-6


def _kernel(gw_hbm, woT_hbm, xT_hbm, wqkv_hbm, bwo_hbm, c_hbm, wq_hbm, wuk_hbm, wuv_hbm,
            oT_hbm,
            xT_sc, wqkv_sc, bwo_sc, c_sc,
            raw_q0, raw_k0, raw_v0, raw_q1, raw_k1, raw_v1,
            pk_q, pk_k, pk_v, ext_q, ext_k, ext_v,
            x_sc, acc_sc, g_sc, wT_sc, bwoT_sc, pqT_sc, gT_sc, kvT_sc, msk_sc, w2_sc, o_sc, gw_sc, woT_sc,
            sems, osems, xsems,
            *, T, H, S, D, M, Dc, HB, TB, CK, AORD, NLATE):
    h = pl.program_id(0)
    scale = D ** -0.5
    Dh = M // HB
    n_t = pl.cdiv(M, 128)
    HG = 8
    PR = HG // 2

    weights = ((wq_hbm, (raw_q0, raw_q1), pk_q, ext_q, M),
               (wuk_hbm, (raw_k0, raw_k1), pk_k, ext_k, Dc),
               (wuv_hbm, (raw_v0, raw_v1), pk_v, ext_v, Dc))

    def w_copy(n, g):
        w_hbm, raws = weights[n][0], weights[n][1]
        return pltpu.make_async_copy(w_hbm.at[:, pl.ds(g * HG, HG), :], raws[g],
                                     sems.at[6 + 3 * g + n])

    WO0 = 2

    def wo_copy(part):
        lo, n, k = (0, WO0, 5) if part == 0 else (WO0, H - WO0, 1)
        return pltpu.make_async_copy(woT_hbm.at[pl.ds(lo, n)], woT_sc.at[pl.ds(lo, n)], sems.at[k])

    def o_copy(i):
        return pltpu.make_async_copy(o_sc.at[:, pl.ds(i * T, T)], oT_hbm.at[:, pl.ds(i * T, T)],
                                     osems.at[i])

    def repack(g):
        CH = 64
        for (_, raws, pk, _, C) in weights:
            def rp(i, carry, raw=raws[g], pk=pk):
                r = pl.multiple_of(i * CH, CH)
                v = raw[pl.ds(r, CH), :, :].reshape(CH // 2, 2 * HG, D)
                u = pltpu.bitcast(v, U32)
                n = CH * PR
                ro = pl.multiple_of(i * n, n)
                for half in range(D // 128):
                    pk[g, half, pl.ds(ro, n), :] = u[:, :, half * 128:(half + 1) * 128].reshape(n, 128)
                return carry
            lax.fori_loop(0, C // CH, rp, 0)

    def extract(hd):
        g = hd // HG
        j = (hd % HG) // 2
        sh = ((hd % 2) * 16).astype(U32)
        for (_, _, pk, ext, C) in weights:
            for half in range(D // 128):
                a = pk[g, half, pl.ds(j, C // 2, stride=2 * PR), :]
                b = pk[g, half, pl.ds(j + PR, C // 2, stride=2 * PR), :]
                r = ((a >> sh) & U32(0xFFFF)) | ((b << (U32(16) - sh)) & U32(0xFFFF0000))
                ext[:, half * 128:(half + 1) * 128] = r

    def trange(t):
        c0, c1 = t * 128, min((t + 1) * 128, M)
        h0, h1 = c0 // Dh, (c1 - 1) // Dh
        r0, r1 = h0 * Dh, (h1 + 1) * Dh
        return c0, c1, (r0 // 16) * 16, min(-(-r1 // 16) * 16, M)

    @pl.when(h == 0)
    def _init():
        cp_wqkv = pltpu.make_async_copy(wqkv_hbm, wqkv_sc, sems.at[0])
        cp_bwo = pltpu.make_async_copy(bwo_hbm, bwo_sc, sems.at[2])
        cp_c = pltpu.make_async_copy(c_hbm, c_sc, sems.at[3])
        cp_gw = pltpu.make_async_copy(gw_hbm, gw_sc, sems.at[4])
        cp_wo = wo_copy(0)

        def x_copy(i):
            r = i * TB if isinstance(i, int) else pl.multiple_of(i * TB, TB)
            return pltpu.make_async_copy(xT_hbm.at[:, pl.ds(r, TB)], xT_sc.at[:, pl.ds(r, TB)],
                                         xsems.at[i])

        cp_wqkv.start()
        cp_gw.start()
        x_copy(0).start()
        ri = lax.broadcasted_iota(jnp.int32, (M, M), 0) // Dh
        ci = lax.broadcasted_iota(jnp.int32, (M, M), 1) // Dh
        msk_sc[0:M, :] = (ri == ci).astype(F32)
        hr = lax.broadcasted_iota(jnp.int32, (HB, M), 0)
        hc = lax.broadcasted_iota(jnp.int32, (HB, M), 1) // Dh
        msk_sc[M:M + HB, :] = (hr == hc).astype(F32)

        kvT_sc[...] = jnp.zeros_like(kvT_sc)
        cp_wqkv.wait()
        for i in range(1, S // TB):
            x_copy(i).start()
        cp_bwo.start()
        cp_gw.wait()
        gw_row = gw_sc[...].reshape(1, M)
        wT_sc[3 * M:3 * M + 16, :] = jnp.broadcast_to(gw_row, (16, M))
        wT_sc[0:3 * M, :] = wqkv_sc[...].T
        cp_c.start()
        for n in range(3):
            w_copy(n, 0).start()
        cp_wo.start()
        ones = jnp.ones((16, TB), BF)
        gw = gw_row.astype(F32)

        def b1(i, carry):
            x_copy(i).wait()
            r = pl.multiple_of(i * TB, TB)
            xTc = xT_sc[:, pl.ds(r, TB)]
            qkvT = _dot(wT_sc[...], xTc)
            pqT_sc[:, pl.ds(r, TB)] = _phi(qkvT[:M]).astype(BF)
            pkT = _phi(qkvT[M:2 * M]).astype(BF)
            vT = qkvT[2 * M:3 * M].astype(BF)
            gT_sc[:, pl.ds(r, TB)] = qkvT[3 * M:3 * M + 8]
            for t in range(n_t):
                c0, c1, r0, r1 = trange(t)
                lhs = jnp.concatenate([vT[r0:r1], ones], axis=0)
                res = _dot_nt(lhs, pkT[c0:c1])
                kvT_sc[r0:r1, c0:c1] += res[:r1 - r0]
                kvT_sc[M:M + 16, c0:c1] += res[r1 - r0:]
            xc = xTc.T
            x_sc[pl.ds(r, TB), :] = xc
            g_sc[pl.ds(r, TB), :] = jax.nn.sigmoid(
                jnp.sum(xc.astype(F32) * gw, axis=-1, keepdims=True))
            return carry

        lax.fori_loop(0, S // TB, b1, 0)

        cp_bwo.wait()
        bwoT_sc[...] = bwo_sc[...].T
        z16 = jnp.where(msk_sc[M:M + HB, :] > 0, kvT_sc[M:M + HB, :], 0.0).astype(BF)
        dens = [_dot(z16, pqT_sc[:, u * TB:(u + 1) * TB]) for u in range(S // TB)]
        for t in range(n_t):
            c0, c1, r0, r1 = trange(t)
            k0, k1 = (r0 // 128) * 128, min(-(-r1 // 128) * 128, M)
            kvm = jnp.where(msk_sc[k0:k1, c0:c1] > 0, kvT_sc[k0:k1, c0:c1], 0.0).astype(BF)
            w2_sc[:, c0:c1] = _dot(bwoT_sc[:, k0:k1], kvm).astype(BF)

        sub8 = lax.broadcasted_iota(jnp.int32, (8, TB), 0)

        def fin(r, den):
            rec = 1.0 / (den + 1e-6)
            pqT = pqT_sc[:, r:r + TB].astype(F32)
            rows = []
            for a in range(0, M, 8):
                h1, h2 = a // Dh, (a + 7) // Dh
                rr = jnp.broadcast_to(rec[h1:h1 + 1], (8, TB))
                if h2 != h1:
                    rr = jnp.where(sub8 < h2 * Dh - a, rr, jnp.broadcast_to(rec[h2:h2 + 1], (8, TB)))
                rows.append(pqT[a:a + 8] * rr)
            pn = jnp.concatenate(rows, axis=0).astype(BF)
            bT = _dot(w2_sc[...], pn)
            gT = jax.nn.sigmoid(gT_sc[0:1, r:r + TB])
            acc_sc[:, r:r + TB] = (1.0 - gT) * bT

        for u in range(S // TB):
            fin(u * TB, dens[u])

        cp_c.wait()
        for n in range(3):
            w_copy(n, 0).wait()
        cp_wo.wait()
        for n in range(3):
            w_copy(n, 1).start()
        wo_copy(1).start()
        repack(0)
        extract(h)

    @pl.when(h == 1)
    def _():
        for n in range(3):
            w_copy(n, 1).wait()
        wo_copy(1).wait()
        repack(1)

    woT = woT_sc[h]
    HT = T // 2
    row = lax.broadcasted_iota(jnp.int32, (HT, HT), 0)
    col = lax.broadcasted_iota(jnp.int32, (HT, HT), 1)
    tri = col <= row
    qs, ks, vs = {}, {}, {}
    state = {}

    def P_(i):
        r0 = i * T
        cch = c_sc[r0:r0 + T, :]
        qs[i] = (_dot(x_sc[r0:r0 + T, :], pltpu.bitcast(ext_q[...], BF)) * scale).astype(BF)
        ks[i] = _dot(cch, pltpu.bitcast(ext_k[...], BF)).astype(BF)
        vs[i] = _dot(cch, pltpu.bitcast(ext_v[...], BF)).astype(BF)

    def kcat(d, a, b):
        parts = []
        t = a // T
        while t * T < b:
            lo, hi = max(a, t * T) - t * T, min(b, (t + 1) * T) - t * T
            parts.append(d[t][lo:hi])
            t += 1
        return jnp.concatenate(parts, axis=0) if len(parts) > 1 else parts[0]

    def S_(i, a, b):
        r0 = i * T
        q = qs[i]
        if b == r0 + T:
            sm = _dot_nt(q, kcat(ks, a, r0 + HT))
            sr = _dot_nt(q[HT:], ks[i][HT:])
            state[(i, a)] = (sm, sr)
        else:
            state[(i, a)] = (_dot_nt(q, kcat(ks, a, b)), None)

    def V_(i, a, b):
        r0 = i * T
        sm, sr = state.pop((i, a))
        if sr is not None:
            w = sm.shape[1]
            dt = jnp.where(tri, sm[:HT, w - HT:], -1e9)
            st = jnp.concatenate([sm[:HT, :w - HT], dt], axis=1) if w > HT else dt
            sb = jnp.concatenate([sm[HT:], jnp.where(tri, sr, -1e9)], axis=1)
            mt = jnp.max(st, axis=-1, keepdims=True)
            mb = jnp.max(sb, axis=-1, keepdims=True)
            pt = jnp.exp(st - mt)
            pb = jnp.exp(sb - mb)
            m = jnp.concatenate([mt, mb], axis=0)
            l = jnp.concatenate([jnp.sum(pt, axis=-1, keepdims=True),
                                 jnp.sum(pb, axis=-1, keepdims=True)], axis=0)
            pb = pb.astype(BF)
            pm = jnp.concatenate([pt.astype(BF), pb[:, :w]], axis=0)
            ctx = _dot(pm, kcat(vs, a, r0 + HT))
            ctx_r = _dot(pb[:, w:], vs[i][HT:])
            ctx = jnp.concatenate([ctx[:HT], ctx[HT:] + ctx_r], axis=0)
        else:
            m = jnp.max(sm, axis=-1, keepdims=True)
            p = jnp.exp(sm - m)
            l = jnp.sum(p, axis=-1, keepdims=True)
            ctx = _dot(p.astype(BF), kcat(vs, a, b))
        state.setdefault(('acc', i), []).append((m, l, ctx))

    def O_(i):
        r0 = i * T
        parts = state.pop(('acc', i))
        m = parts[0][0]
        for (mc, _, _) in parts[1:]:
            m = jnp.maximum(m, mc)
        if len(parts) == 1:
            rr = g_sc[r0:r0 + T, :] / parts[0][1]
            ctx = parts[0][2] * rr
        else:
            es = [jnp.exp(mc - m) for (mc, _, _) in parts]
            l = sum(e * lc for e, (_, lc, _) in zip(es, parts))
            rr = g_sc[r0:r0 + T, :] / l
            ctx = sum((e * rr) * cx for e, (_, _, cx) in zip(es, parts))
        a_new = acc_sc[:, r0:r0 + T] + _dot_nt(woT, ctx.astype(BF))
        acc_sc[:, r0:r0 + T] = a_new
        o_sc[:, r0:r0 + T] = a_new.astype(BF)
        if i not in AORD[-NLATE:]:
            o_copy(i).start()

    items = []
    donep = 0
    for i in AORD:
        while donep <= i:
            items.append(('P', donep))
            donep += 1
        end = (i + 1) * T
        bnds = list(range(0, end, CK)) + [end]
        for a, b in zip(bnds[:-1], bnds[1:]):
            items.append(('S', i, a, b))
    out = []
    pend_v = []
    pend_o = []

    def emit(x):
        out.append(x)
        if pend_o:
            out.append(pend_o.pop(0))

    def emit_v(x):
        emit(('V',) + x[1:])
        if x[3] == (x[1] + 1) * T:
            pend_o.append(('O', x[1]))

    for it in items:
        emit(it)
        if pend_v:
            emit_v(pend_v.pop(0))
        if it[0] == 'S':
            pend_v.append(it)
    while pend_v:
        emit_v(pend_v.pop(0))
    out.extend(pend_o)
    for it in out:
        {'P': P_, 'S': S_, 'V': V_, 'O': O_}[it[0]](*it[1:])

    extract(jnp.minimum(h + 1, H - 1))

    for i in AORD[:-NLATE]:
        o_copy(i).wait()

    @pl.when(h == H - 1)
    def _():
        for i in AORD[-NLATE:]:
            o_copy(i).start()
        for i in AORD[-NLATE:]:
            o_copy(i).wait()


@jax.jit
def pallas_gated_mix__compressed_kv_cla__linear_attn_block__prompt_kernel(
    A_x: jax.Array,
    A_c_kv: jax.Array,
    A_w_q: jax.Array,
    A_w_uk: jax.Array,
    A_w_uv: jax.Array,
    A_w_o: jax.Array,
    B_x: jax.Array,
    B_wqkv: jax.Array,
    B_wo: jax.Array,
    gate_w: jax.Array,
):
    B, S, M = A_x.shape
    Dc = A_c_kv.shape[2]
    H, D = A_w_q.shape[1], A_w_q.shape[2]
    assert B == 1 and A_c_kv.shape[1] == S and H == 16 and D == 256 and S == 2048
    T = 256
    TB = 512
    HB = 16
    CK = 512
    AORD = (1, 3, 4, 5, 6, 7, 2, 0)
    NLATE = 2
    xT = jnp.swapaxes(A_x, 1, 2).reshape(M, S)
    woT = jnp.swapaxes(A_w_o, 1, 2)
    c = A_c_kv.reshape(S, Dc)
    kern = functools.partial(_kernel, T=T, H=H, S=S, D=D, M=M, Dc=Dc, HB=HB, TB=TB, CK=CK,
                             AORD=AORD, NLATE=NLATE)
    hbm_spec = pl.BlockSpec(memory_space=pltpu.MemorySpace.HBM)
    NG = H // 8
    outT = pl.pallas_call(
        kern,
        grid=(H,),
        in_specs=[hbm_spec] * 9,
        out_specs=hbm_spec,
        out_shape=jax.ShapeDtypeStruct((M, S), BF),
        scratch_shapes=[
            pltpu.VMEM((M, S), BF),
            pltpu.VMEM((M, 3 * M), BF),
            pltpu.VMEM((M, M), BF),
            pltpu.VMEM((S, Dc), BF),
            pltpu.VMEM((M, 8, D), BF),
            pltpu.VMEM((Dc, 8, D), BF),
            pltpu.VMEM((Dc, 8, D), BF),
            pltpu.VMEM((M, 8, D), BF),
            pltpu.VMEM((Dc, 8, D), BF),
            pltpu.VMEM((Dc, 8, D), BF),
            pltpu.VMEM((NG, D // 128, M * 4 + 8, 128), U32),
            pltpu.VMEM((NG, D // 128, Dc * 4 + 8, 128), U32),
            pltpu.VMEM((NG, D // 128, Dc * 4 + 8, 128), U32),
            pltpu.VMEM((M // 2, D), U32),
            pltpu.VMEM((Dc // 2, D), U32),
            pltpu.VMEM((Dc // 2, D), U32),
            pltpu.VMEM((S, M), BF),
            pltpu.VMEM((M, S), F32),
            pltpu.VMEM((S, 1), F32),
            pltpu.VMEM((3 * M + 16, M), BF),
            pltpu.VMEM((M, M), BF),
            pltpu.VMEM((M, S), BF),
            pltpu.VMEM((8, S), F32),
            pltpu.VMEM((M + 16, M), F32),
            pltpu.VMEM((M + HB, M), F32),
            pltpu.VMEM((M, M), BF),
            pltpu.VMEM((M, S), BF),
            pltpu.VMEM((M,), BF),
            pltpu.VMEM((H, M, D), BF),
            pltpu.SemaphoreType.DMA((6 + 3 * NG,)),
            pltpu.SemaphoreType.DMA((S // T,)),
            pltpu.SemaphoreType.DMA((S // TB,)),
        ],
        compiler_params=pltpu.CompilerParams(
            dimension_semantics=("arbitrary",),
            vmem_limit_bytes=110 * 1024 * 1024),
    )(gate_w, woT, xT, B_wqkv, B_wo, c, A_w_q, A_w_uk, A_w_uv)
    return jnp.swapaxes(outT.reshape(B, M, S), 1, 2)
```
